```python
import os as _os
_os.environ.setdefault("JAX_PLATFORMS", "cpu")
import jax
import jax.numpy as jnp

def _softmax(x, axis=-1):
    return jax.nn.softmax(x, axis=axis)
def _gelu(x):
    return jax.nn.gelu(x, approximate=True)
def _silu(x):
    return jax.nn.silu(x)
def _sigmoid(x):
    return jax.nn.sigmoid(x)
def _layernorm(x, axis=-1, eps=1e-5):
    m = jnp.mean(x, axis=axis, keepdims=True)
    v = jnp.var(x, axis=axis, keepdims=True)
    return (x - m) / jnp.sqrt(v + eps)
def _scatter_add(tgt, idx, src, axis=0):
    return tgt.at[idx].add(src)
def _segment_sum(src, seg, n):
    return jax.ops.segment_sum(src, seg, n)
class _Rng:
    def __init__(self, key):
        self._k = key
    def _next(self):
        self._k, sub = jax.random.split(self._k)
        return sub
    def normal(self, shape):
        return jax.random.normal(self._next(), shape, dtype=jnp.bfloat16)
    def randint(self, lo, hi, shape):
        return jax.random.randint(self._next(), shape, lo, hi, dtype=jnp.int32)
    def uniform(self, shape, lo=0.0, hi=1.0):
        return jax.random.uniform(self._next(), shape, jnp.bfloat16, lo, hi)
    def permutation(self, n):
        return jax.random.permutation(self._next(), n)


kernel_name = 'standalone__gqa_block_cached__near_ridge'

def setup_inputs():
    _rng = _Rng(jax.random.key(int.from_bytes(__import__("os").urandom(4), "little")))
    _w = (lambda a: (lambda t: t.astype(jnp.bfloat16) if jnp.issubdtype(t.dtype, jnp.floating) else t)(jnp.asarray(a)))
    B, Sq, D = 8, 240, 640
    Hq, Hkv, Sk, Dh = 32, 32, 1024, 192
    assert Hq % Hkv == 0, (Hq, Hkv)
    return {
        "x": _w((lambda *s: _rng.normal(s) * 0.8)(B, Sq, D)),
        "k_cache": _w((lambda *s: _rng.normal(s) * 0.8)(B, Hkv, Sk, Dh)),
        "v_cache": _w((lambda *s: _rng.normal(s) * 0.05)(B, Hkv, Sk, Dh)),
        "wq": _w((lambda *s: _rng.normal(s) * 0.8)(D, Hq * Dh) * (D ** -0.5)),
        "wo": _w((lambda *s: _rng.normal(s) * 0.05)(Hq * Dh, D) * ((Hq * Dh) ** -0.5)),
    }

def reference(x, k_cache, v_cache, wq, wo):
    B, Sq, D = x.shape
    Hq, Dh = 32, 192
    Hkv = k_cache.shape[1]
    rep = Hq // Hkv
    q = (lambda x, *d: x.transpose(*d))((x @ wq).reshape(B, Sq, Hq, Dh), 0, 2, 1, 3)
    k = jnp.repeat(k_cache, rep, axis=1)
    v = jnp.repeat(v_cache, rep, axis=1)
    scores = jnp.einsum("bhqd,bhkd->bhqk", q, k) * (Dh ** -0.5)
    p = _softmax(scores, axis=-1)
    o = jnp.einsum("bhqk,bhkd->bhqd", p, v)
    return (lambda x, *d: x.transpose(*d))(o, 0, 2, 1, 3).reshape(B, Sq, Hq * Dh) @ wo
```

```python
import math, re
import jax, jax.numpy as jnp
from jax import lax
import jax.experimental.pallas as pl
import jax.experimental.pallas.tpu as pltpu

F32 = jnp.float32
BF16 = jnp.bfloat16
U32 = jnp.uint32
ORDER4 = "t0 t1 q00 q01 o0 s0 q02 q10 o1 s1 pv0 q11 q12 o2 s2 s3 pv1 o3 o4 pv2 pv3"
LAST4 = "t0 t1 q00 q01 o0 s0 q02 q10 o1 s1 pv0 q11 q12 o2 s2 s3 pv1 o3 o4 F t0 pv2 pv3 H0 t1 H1"
FIRSTQ = "s0 s1 s2 s3 pv0 pv1 pv2 pv3"
NOQ4 = "t0 t1 s0 o0 o1 s1 pv0 s2 s3 pv1 o2 o3 o4 pv2 pv3"

def parse(order):
    return [(re.match(r"[a-zA-Z]+", t).group(0), (re.search(r"\d+", t) or [""])[0]) for t in order.split()]

def _run(x, k_cache, v_cache, wq, wo, HB=4, RC=16, pvs='LAB', rat=0, nqa=4, dly=4, ocut=(2, 4, 5)):
    B, Sq, D = x.shape
    _, H, Sk, Dh = k_cache.shape
    kT = jnp.swapaxes(k_cache, 2, 3)
    vT = jnp.swapaxes(v_cache, 2, 3)
    scale = (Dh ** -0.5) * math.log2(math.e)
    NG = H // HB
    NP = HB // 2
    NIT = NG * B
    C = Dh // 3; RA = 128; RB = Sq - RA
    NT = Sk // 128; PR = Sq // 2; NR = Sq // RC; ND = D // 128
    GW = HB * Dh
    QP = D // B
    OP = GW // B
    SP = 256
    order = parse(ORDER4); first = parse(FIRSTQ); lo = B; ocut = list(ocut)

    def kernel(x_hbm, kT_hbm, vT_hbm, wq_hbm, wo_hbm, o_hbm, xbuf, kbuf, vbuf, wqbuf, wobuf, obuf, acc_ref,
               sem_x, sem_k, sem_v, sem_w, sem_o, sem_f, *scr):
        l_refs = scr[0:HB]; s_refs = scr[HB:2*HB]; m_refs = scr[2*HB:3*HB]; p_refs = scr[3*HB:4*HB]
        r_refs = scr[4*HB:5*HB]; ob_refs = scr[5*HB:5*HB+NP]; pb_refs = scr[5*HB+NP:6*HB+NP]; on_refs = scr[6*HB+NP:7*HB+NP]; xpk = scr[7*HB+NP]
        L1, L2, L3 = slice(0, 64), slice(64, 128), slice(128, 128 + RB // 2)
        LO, HI = slice(0, C), slice(C, 128)
        def dot(a, w): return jnp.dot(a, w, preferred_element_type=F32)
        cat = lambda u, v: jnp.concatenate([u, v], axis=0)
        pk = lambda v: pltpu.bitcast(v.astype(BF16), U32)
        upk = lambda v: pltpu.bitcast(v, BF16)

        LB = B.bit_length() - 1
        def divB(v): return v // B if isinstance(v, int) else lax.shift_right_logical(v, LB)
        def remB(v): return v % B if isinstance(v, int) else v & (B - 1)
        def rem2(v): return v % 2 if isinstance(v, int) else v & 1
        def mn(v, c): return min(v, c) if isinstance(v, int) else jnp.minimum(v, c)
        def mul(v, c): return v if isinstance(v, int) else pl.multiple_of(v, c)
        def make(i, lb=False):
            if isinstance(i, int): z1 = z2 = z3 = 0
            else:
                z1 = lax.shift_right_logical(i, 20); z2 = lax.shift_right_logical(i, 21); z3 = lax.shift_right_logical(i, 22)
            zs = [z1, z2, z3]
            lw = (remB(i) if lb else z1); lr_ = (remB(i) if lb else z2)
            slot = rem2(i); grp = divB(i); ip = i - 1; bprev = remB(i + (B - 1))
            def cp_k(it, sl): return pltpu.make_async_copy(kT_hbm.at[remB(it), pl.ds(divB(it) * HB, HB)], kbuf.at[sl], sem_k.at[sl])
            def cp_v(it, sl): return pltpu.make_async_copy(vT_hbm.at[remB(it), pl.ds(divB(it) * HB, HB)], vbuf.at[sl], sem_v.at[sl])
            def cp_wq(it):
                g = divB(it) + 1
                r0 = mul(remB(it) * QP, QP)
                c0 = mul(mn(g, NG - 1) * GW, GW)
                return pltpu.make_async_copy(wq_hbm.at[pl.ds(r0, QP), pl.ds(c0, GW)], wqbuf.at[rem2(g), pl.ds(r0, QP)], sem_w.at[rem2(it)])
            def cp_wo(it):
                j = it + (B - 1)
                g = divB(j)
                r0 = mul(remB(j) * OP, OP)
                s0 = mul(mn(g, NG - 1) * GW + r0, OP)
                return pltpu.make_async_copy(wo_hbm.at[pl.ds(s0, OP)], wobuf.at[rem2(g), pl.ds(r0, OP)], sem_w.at[2 + rem2(it)])
            def cp_out(bb): return pltpu.make_async_copy(obuf.at[bb], o_hbm.at[bb], sem_o.at[bb])
            def cp_fin(c):
                cs = pl.ds(128 * ([0] + ocut)[c], 128 * (ocut[c] - ([0] + ocut)[c]))
                return pltpu.make_async_copy(obuf.at[B - 1, :, cs], o_hbm.at[B - 1, :, cs], sem_o.at[B - 1 + c])
            def start_for(it):
                nx = mn(it + 1, NIT - 1); sl = rem2(it + 1)
                cp_k(nx, sl).start(); cp_v(nx, sl).start()
                cp_wo(it).start(); cp_wq(it).start()
            def wait_for(it):
                sl = rem2(it); cu = mn(it, NIT - 1)
                cp_k(cu, sl).wait(); cp_v(cu, sl).wait()
                cp_wo(it - 1).wait(); cp_wq(it - 1).wait()
            def tail():
                start_for(i + 1)

            def recip(h):
                tot = jnp.broadcast_to(jnp.sum(m_refs[h][z2, Dh:, 128:], axis=1, keepdims=True), (Sq, 128))
                r = pl.reciprocal(tot, approx=True)
                return r * (2.0 - tot * r)

            def prep(p):
                r0 = r_refs[2*p][z2, :Sq]; r1 = r_refs[2*p+1][z2, :Sq]
                lo = lax.broadcasted_iota(jnp.int32, (Sq, 128), 1) < C
                t = cat(m_refs[2*p][z2, :C, :Sq], m_refs[2*p+1][z2, :C, :Sq]).T
                o = jnp.concatenate([on_refs[2*p][z2, :Sq] * r0, on_refs[2*p+1][z2, :Sq] * r1, t * jnp.where(lo, r0, r1)], axis=1)
                ob_refs[p][z1, :PR] = pk(o)

            def wo_rows(ws, p, n):
                cs = slice(n*128, (n+1)*128); b0 = p*2*Dh
                g = lambda u, v: wobuf[ws, b0 + u:b0 + v, cs]
                return jnp.concatenate([g(0, 128), g(Dh, Dh + 128), g(128, Dh), g(Dh + 128, 2*Dh)], axis=0)

            def ogroup(n, cur=False):
                o = jnp.concatenate([upk(ob_refs[p][z2, :PR]) for p in range(NP)], axis=1)
                wslot = rem2(divB(i if cur else ip))
                acc_ref[remB(i) if cur else bprev, :Sq, n*128:(n+1)*128] += dot(o, jnp.concatenate([wo_rows(wslot, p, n) for p in range(NP)], axis=0))
            def ohalf(p):
                o = upk(ob_refs[p][z2, :PR])
                for n in range(ND):
                    cs = slice(n*128, (n+1)*128)
                    v = acc_ref[remB(i), :Sq, cs] + dot(o, wo_rows(rem2(divB(i)), p, n))
                    if p + 1 < NP: acc_ref[remB(i), :Sq, cs] = v
                    else:
                        obuf[B - 1, :, cs] = v.astype(obuf.dtype)
                        if n + 1 in ocut: cp_fin(ocut.index(n + 1)).start()

            def qgroup(p, j):
                lo_a = lax.broadcasted_iota(jnp.int32, (RA, 128), 1) < C
                if lb and (p, j) == (0, 0): xpk[remB(i), :Sq//2] = pk(xbuf[remB(i), :Sq])
                xv = xbuf[remB(i) + zs[j], :Sq] if lb else upk(xpk[remB(i) + zs[j], :Sq//2])
                t = dot(xv, wqbuf[rem2(grp), :, p*2*Dh + j*128:p*2*Dh + (j+1)*128]) * scale
                tA = t[:RA]; tB = t[RA:]
                le, lod = l_refs[2*p], l_refs[2*p+1]
                if j == 1:
                    a = pk(tA); rb = pk(pltpu.roll(tB, C, 1))
                    le[lw, L2, LO] = a[:, LO]; lod[lw, L2, HI] = a[:, HI]
                    le[lw, L3, HI] = rb[:, HI]; lod[lw, L3, LO] = rb[:, LO]
                else:
                    tBp = cat(tB, jnp.zeros((RA - RB, 128), F32))
                    if j == 0:
                        l1 = jnp.where(lo_a, tA, tBp).astype(BF16)
                        d = pk(jnp.where(lo_a, tBp, tA) - l1.astype(F32))
                        le[lw, L1, :] = pltpu.bitcast(l1, U32)
                        le[lw, L2, HI] = d[:, HI]; le[lw, L3, LO] = d[:RB//2, LO]
                    else:
                        l1 = jnp.where(lo_a, tBp, tA).astype(BF16)
                        d = pk(jnp.where(lo_a, tA, tBp) - l1.astype(F32))
                        lod[lw, L1, :] = pltpu.bitcast(l1, U32)
                        lod[lw, L2, LO] = d[:, LO]; lod[lw, L3, HI] = d[:RB//2, HI]

            def scores(h):
                lr = l_refs[h]; sr = s_refs[h]; mr = m_refs[h]; pr = p_refs[h]
                for j in range(NT):
                    cs = slice(j*128, (j+1)*128)
                    kc = lambda c: kbuf[slot, h, c*C:(c+1)*C, cs]
                    if h % 2 == 0:
                        w1, w2, w3 = kbuf[slot, h, 0:2*C, cs], cat(kc(2), kc(1)), cat(kc(0), kc(2))
                    else:
                        w1, w2, w3 = kbuf[slot, h, C:3*C, cs], cat(kc(1), kc(0)), cat(kc(0), kc(2))
                    c1 = dot(upk(lr[lr_, L1]), w1)
                    c2 = dot(upk(lr[lr_, L2]), w2)
                    c3 = dot(upk(lr[lr_, L3]), w3)
                    sr[z1, :RA, cs] = c1 + c2
                    sr[z1, RA:, cs] = c1[:RB] + c3
            def softmax(h):
                sr = s_refs[h]; mr = m_refs[h]; pr = p_refs[h]
                for r in range(NR):
                    m = jnp.max(sr[z2, r*RC:(r+1)*RC, :], axis=1, keepdims=True)
                    mr[z1, Dh + r*RC:Dh + (r+1)*RC, :128] = jnp.broadcast_to(m, (RC, 128))
                for r in range(NR):
                    rs = slice(r*RC, (r+1)*RC)
                    m = mr[z2, Dh + r*RC:Dh + (r+1)*RC, :128]
                    p = sr[z3, rs, :] - jnp.tile(m, (1, NT))
                    p = jnp.exp2(p)
                    part = p[:, 0:128]
                    for t in range(1, NT): part = part + p[:, t*128:(t+1)*128]
                    if r + 1 == NR or (r + 1) * RC == RA:
                        plast = jnp.minimum(p[:, (NT-1)*128:], part)
                        p = jnp.concatenate([p[:, :(NT-1)*128], plast], axis=1)
                    if rs.start < RA: pr[z1, rs.start//2:rs.stop//2, :] = pk(p)
                    else: pb_refs[h][z1, (rs.start - RA)//2:(rs.stop - RA)//2, :] = pk(p)
                    mr[z1, Dh + r*RC:Dh + (r+1)*RC, 128:] = part

            def pv(h, last=False):
                nt = (((1,), (1,)), ((), ()))
                ntd = lambda u, w: lax.dot_general(u, w, nt, preferred_element_type=F32)
                KH = Sk // 2
                acc = {}
                steps = [(c, kk) for kk in range(2) for c in pvs]
                for sn, (c, kk) in enumerate(steps):
                    ks = slice(kk*KH, (kk+1)*KH)
                    zz = z2 if c == 'L' else z3
                    pa = lambda: upk(p_refs[h][zz, :, ks]); pb = lambda: upk(pb_refs[h][zz, :, ks])
                    if c == 'L': v = ntd(cat(pa(), pb()), vbuf[slot, h, :128, ks])
                    else: v = ntd(vbuf[slot + (z1 if c == 'A' else z2), h, 128:, ks], pa() if c == 'A' else pb())
                    if last and sn == len(steps) - 1: tail()
                    if c == 'L':
                        if kk == 0: on_refs[h][z1, :Sq] = v
                        else: on_refs[h][z1, :Sq] = on_refs[h][z3, :Sq] + v
                    elif kk == 0: acc[c] = v
                    else: m_refs[h][z1, :C, (slice(0, RA) if c == 'A' else slice(RA, Sq))] = acc[c] + v
                    if sn == rat:
                        m_refs[h][z1, C:C+8, :v.shape[1]] = v[:8]
                        r_refs[h][z1, :Sq] = recip(h)

            def emit(tokens, dma=True):
                for n, (kind, arg) in enumerate(tokens):
                    if kind == "q": qgroup(int(arg[0]), int(arg[1]))
                    elif kind == "s": scores(int(arg)); softmax(int(arg))
                    elif kind == "S": scores(int(arg))
                    elif kind == "m": softmax(int(arg))
                    elif kind == "pv": pv(int(arg), last=(dma and n == len(tokens) - 1))
                    elif kind == "t": prep(int(arg))
                    elif kind == "o": ogroup(int(arg))
                    elif kind == "O": ogroup(int(arg), cur=True)
                    elif kind == "H": ohalf(int(arg))
                    elif kind == "F": flush(bprev)

            def flush(bb):
                obuf[bb] = acc_ref[bb, :Sq].astype(obuf.dtype)
                cp_out(bb).start()

            return dict(cp_k=cp_k, cp_v=cp_v, wait_for=wait_for, emit=emit, flush=flush, start_for=start_for, prep=prep, ogroup=ogroup, cp_out=cp_out, cp_fin=cp_fin, bprev=bprev)

        f0 = make(0)
        def cp_x(bb): return pltpu.make_async_copy(x_hbm.at[bb], xbuf.at[bb, pl.ds(0, Sq)], sem_x.at[bb])
        cuts = (0, nqa * 128, GW)
        wq0 = [pltpu.make_async_copy(wq_hbm.at[:, pl.ds(cuts[c], cuts[c + 1] - cuts[c])], wqbuf.at[0, :, pl.ds(cuts[c], cuts[c + 1] - cuts[c])], sem_f.at[2 * c]) for c in range(2)]
        bulk = pltpu.make_async_copy(wo_hbm.at[pl.ds(0, GW - OP)], wobuf.at[0, pl.ds(0, GW - OP)], sem_f.at[1])
        cp_x(0).start(); wq0[0].start()
        acc_ref[:, :Sq] = jnp.zeros((B, Sq, D), F32)
        qtoks = [("q", f"{p}{j}") for p in range(NP) for j in range(3)]
        wq0[1].start(); cp_x(1).start()
        cp_x(0).wait(); wq0[0].wait()
        for bb in range(2, dly): cp_x(bb).start()
        make(0, lb=True)["emit"](qtoks[:nqa], dma=False)
        wq0[1].wait(); cp_x(1).wait()
        for bb in range(dly, B): cp_x(bb).start()
        f0["cp_k"](0, 0).start(); f0["cp_v"](0, 0).start()
        f0["start_for"](0)
        bulk.start()
        make(0, lb=True)["emit"](qtoks[nqa:], dma=False)
        make(1, lb=True)["emit"](qtoks, dma=False)
        def qstep(j, carry):
            cp_x(2 * j).wait(); cp_x(2 * j + 1).wait()
            make(2 * j, lb=True)["emit"](qtoks, dma=False)
            make(2 * j + 1, lb=True)["emit"](qtoks, dma=False)
            return carry + j
        nj = B // 2
        i0 = lax.fori_loop(1, nj, qstep, 0) - sum(range(1, nj))
        f0["cp_k"](0, 0).wait(); f0["cp_v"](0, 0).wait()
        make(i0, lb=True)["emit"](first)
        bulk.wait()
        def nstep(i, carry):
            f = make(i, lb=True)
            f["wait_for"](i)
            f["emit"](parse(NOQ4))
            return carry
        lax.fori_loop(1, B, nstep, 0)

        def step(i, carry):
            f = make(i)
            f["wait_for"](i)
            f["emit"](order)
            @pl.when(i > NIT - B)
            def _():
                f["flush"](f["bprev"])
            return carry + i
        tot = lax.fori_loop(lo, NIT - 1, step, 0)
        il = tot - (sum(range(lo, NIT - 1)) - (NIT - 1))
        fe = make(il)
        fe["wait_for"](NIT - 1)
        fe["emit"](parse(LAST4), dma=False)
        fe["wait_for"](NIT)
        for bb in range(B - 1): fe["cp_out"](bb).wait()
        for c in range(len(ocut)): fe["cp_fin"](c).wait()

    any_spec = pl.BlockSpec(memory_space=pl.ANY)
    return pl.pallas_call(
        kernel,
        in_specs=[any_spec] * 5,
        out_specs=any_spec,
        out_shape=jax.ShapeDtypeStruct((B, Sq, D), x.dtype),
        scratch_shapes=[pltpu.VMEM((B, SP, D), BF16), pltpu.VMEM((2, HB, Dh, Sk), BF16), pltpu.VMEM((2, HB, Dh, Sk), BF16),
                        pltpu.VMEM((2, D, GW), BF16), pltpu.VMEM((2, GW, D), BF16),
                        pltpu.VMEM((B, Sq, D), BF16),
                        pltpu.VMEM((B, SP, D), F32),
                        pltpu.SemaphoreType.DMA((B,)), pltpu.SemaphoreType.DMA((2,)), pltpu.SemaphoreType.DMA((2,)),
                        pltpu.SemaphoreType.DMA((4,)), pltpu.SemaphoreType.DMA((B - 1 + len(ocut),)),
                        pltpu.SemaphoreType.DMA((3,)),
                        *[pltpu.VMEM((B, 192, 128), U32)]*HB,
                        *[pltpu.VMEM((1, Sq, Sk), F32)]*HB,
                        *[pltpu.VMEM((1, Dh + Sq, 256), F32)]*HB,
                        *[pltpu.VMEM((1, RA // 2, Sk), U32)]*HB,
                        *[pltpu.VMEM((1, SP, 128), F32)]*HB,
                        *[pltpu.VMEM((1, SP // 2, 2*Dh), U32)]*NP,
                        *[pltpu.VMEM((1, RB // 2, Sk), U32)]*HB,
                        *[pltpu.VMEM((1, SP, 128), F32)]*HB,
                        pltpu.VMEM((B, SP // 2, D), U32),
                        ],
        compiler_params=pltpu.CompilerParams(vmem_limit_bytes=100*1024*1024),
    )(x, kT, vT, wq, wo)


@jax.jit
def pallas_standalone__gqa_block_cached__near_ridge_kernel(x, k_cache, v_cache, wq, wo):
    return _run(x, k_cache, v_cache, wq, wo)
```
